```python
import os as _os
_os.environ.setdefault("JAX_PLATFORMS", "cpu")
import jax
import jax.numpy as jnp

def _softmax(x, axis=-1):
    return jax.nn.softmax(x, axis=axis)
def _gelu(x):
    return jax.nn.gelu(x, approximate=True)
def _silu(x):
    return jax.nn.silu(x)
def _sigmoid(x):
    return jax.nn.sigmoid(x)
def _layernorm(x, axis=-1, eps=1e-5):
    m = jnp.mean(x, axis=axis, keepdims=True)
    v = jnp.var(x, axis=axis, keepdims=True)
    return (x - m) / jnp.sqrt(v + eps)
def _scatter_add(tgt, idx, src, axis=0):
    return tgt.at[idx].add(src)
def _segment_sum(src, seg, n):
    return jax.ops.segment_sum(src, seg, n)
class _Rng:
    def __init__(self, key):
        self._k = key
    def _next(self):
        self._k, sub = jax.random.split(self._k)
        return sub
    def normal(self, shape):
        return jax.random.normal(self._next(), shape, dtype=jnp.bfloat16)
    def randint(self, lo, hi, shape):
        return jax.random.randint(self._next(), shape, lo, hi, dtype=jnp.int32)
    def uniform(self, shape, lo=0.0, hi=1.0):
        return jax.random.uniform(self._next(), shape, jnp.bfloat16, lo, hi)
    def permutation(self, n):
        return jax.random.permutation(self._next(), n)


kernel_name = 'sequential_preLN__mha_block__moe_arch_mod__prompt'

def setup_inputs():
    _rng = _Rng(jax.random.key(int.from_bytes(__import__("os").urandom(4), "little")))
    _w = (lambda a: (lambda t: t.astype(jnp.bfloat16) if jnp.issubdtype(t.dtype, jnp.floating) else t)(jnp.asarray(a)))
    def _A_setup():
        B, S, D, H = 1, 2048, 512, 32
        return {
            "x": _w((lambda *s: _rng.normal(s) * 0.05)(B, S, D)),
            "wqkv": _w((lambda *s: _rng.normal(s) * 0.05)(D, 3 * D)),
            "wo": _w((lambda *s: _rng.normal(s) * 0.05)(D, D)),
        }
    _A_in = _A_setup()

    def _B_setup():
        B, S, D, F, C = 1, 2048, 512, 1792, 2
        return {
            "x": _w((lambda *s: _rng.normal(s) * 0.05)(B, S, D)),
            "w_r": _w((lambda *s: _rng.normal(s) * 0.05)(D)),
            "w_gate": _w((lambda *s: _rng.normal(s) * 0.05)(D, F)),
            "w_up": _w((lambda *s: _rng.normal(s) * 0.05)(D, F)),
            "w_down": _w((lambda *s: _rng.normal(s) * 0.05)(F, D)),
        }
    _B_in = _B_setup()

    return {
        "A_x": _A_in["x"],
        "A_wqkv": _A_in["wqkv"],
        "A_wo": _A_in["wo"],
        "B_x": _B_in["x"],
        "B_w_r": _B_in["w_r"],
        "B_w_gate": _B_in["w_gate"],
        "B_w_up": _B_in["w_up"],
        "B_w_down": _B_in["w_down"],
    }

def reference(A_x, A_wqkv, A_wo, B_x, B_w_r, B_w_gate, B_w_up, B_w_down):
    def _A_ref(x, wqkv, wo):
        B, S, D = x.shape
        H = 32
        Dh = D // H
        qkv = (lambda x, *d: x.transpose(*d))((x @ wqkv).reshape(B, S, 3, H, Dh), 2, 0, 3, 1, 4)
        q, k, v = qkv[0], qkv[1], qkv[2]
        scores = jnp.einsum("bhqd,bhkd->bhqk", q, k) * (Dh ** -0.5)
        p = _softmax(scores, axis=-1)
        o = jnp.einsum("bhqk,bhkd->bhqd", p, v)
        return (lambda x, *d: x.transpose(*d))(o, 0, 2, 1, 3).reshape(B, S, D) @ wo

    def _B_ref(x, w_r, w_gate, w_up, w_down):
        B, S, D = x.shape
        C = 2
        r = x @ w_r
        idx = jnp.argsort(-r, axis=-1)[:, :C]
        idx_e = jnp.repeat(idx.reshape(B, C, 1), D, axis=2)
        x_sel = jnp.take_along_axis(x, idx_e, axis=1)
        g = _silu(x_sel @ w_gate)
        u = x_sel @ w_up
        y = (g * u) @ w_down
        r_sel = _sigmoid(jnp.take_along_axis(r, idx, axis=1))
        y = y * r_sel.reshape(B, C, 1)
        b_off = (jnp.arange(B) * S).reshape(B, 1)
        flat_idx = (idx + b_off).reshape(B * C)
        zero = (x * 0.0).reshape(B * S, D)
        upd = _scatter_add(zero, flat_idx, y.reshape(B * C, D), axis=0)
        return x + upd.reshape(B, S, D)

    x = A_x
    h = x + _A_ref(_layernorm(x, axis=-1), A_wqkv, A_wo)
    h2 = h + _B_ref(_layernorm(h, axis=-1), B_w_r, B_w_gate, B_w_up, B_w_down)
    return h2
```

```python
import functools

import jax
import jax.numpy as jnp
import numpy as np
from jax import lax
from jax.experimental import pallas as pl
from jax.experimental.pallas import tpu as pltpu

F32, BF16, U32, I32 = jnp.float32, jnp.bfloat16, jnp.uint32, jnp.int32

NUM_HEADS = 32
HEAD_DIM = 16
CAPACITY = 2
LN_EPS = 1e-5

TQ = 512
CK = 128
ROWS_OUT = 256

SUM_LO, SUM_HI = 2.0**-30, 2.0**30

CFG = dict(off=1, tie=(0, 1, 3, 5), nacc=4, hb=2, nocse=True, kbtie=True, vlook=1)

NT = (((1,), (1,)), ((), ()))
NN = (((1,), (0,)), ((), ()))
TN = (((0,), (0,)), ((), ()))


def _dot(a, b, dims=NN):
    return lax.dot_general(a, b, dims, preferred_element_type=F32)


def _rnd(x):
    return x.astype(BF16).astype(F32)


def _pack(x):
    return pltpu.bitcast(x.astype(BF16), U32)


def _unpack(x):
    return pltpu.bitcast(x, BF16)


def _layernorm(x):
    mean = jnp.mean(x, axis=-1, keepdims=True)
    centered = x - mean
    var = jnp.mean(centered * centered, axis=-1, keepdims=True)
    std = _rnd(jnp.sqrt(_rnd(_rnd(var) + LN_EPS)))
    return (_rnd(x - _rnd(mean)) * (1.0 / std)).astype(BF16)


def _sum_tree(terms, lanes):
    accs = list(terms[:lanes])
    for i, t in enumerate(terms[lanes:]):
        accs[i % lanes] = accs[i % lanes] + t
    while len(accs) > 1:
        accs = [accs[i] + accs[i + 1] for i in range(0, len(accs), 2)]
    return accs[0]


def _kernel(
    x_hbm, wqkv_hbm, wo_hbm, wr_ref, wg_hbm, wu_hbm, wd_hbm,
    out_hbm,
    x_v, wqkv_v, wo_v, wg_v, wu_v, wd_v,
    wt_v, qt_v, kk_v, vt_v, kba_v, kbb_v, ot_v,
    h_v, hn_v, out_v, fix_v,
    in_sem, out_sem, fix_sem,
    *, cfg,
):
    seq, dim = x_v.shape
    n_qb = seq // TQ
    n_ck = seq // CK
    n_col = TQ // 128
    q_scale = HEAD_DIM**-0.5 * np.log2(np.e)

    def x_copy(i):
        rows = pl.ds(pl.multiple_of(i * TQ, TQ), TQ)
        return pltpu.make_async_copy(x_hbm.at[0, rows], x_v.at[rows], in_sem.at[i])

    def w_copy(j):
        cols = pl.ds(j * dim, dim)
        return pltpu.make_async_copy(wqkv_hbm.at[:, cols], wqkv_v.at[:, cols], in_sem.at[n_qb + j])

    late = [
        pltpu.make_async_copy(src, dst, in_sem.at[n_qb + 3 + j])
        for j, (src, dst) in enumerate(
            [(wo_hbm, wo_v), (wg_hbm, wg_v), (wu_hbm, wu_v), (wd_hbm, wd_v)])
    ]
    x_copy(0).start()
    for j in (0, 2, 1):
        w_copy(j).start()
    for i in range(1, n_qb):
        x_copy(i).start()

    w_copy(0).wait()
    wt_v[0:dim, :] = wqkv_v[:, 0:dim].T
    w_copy(2).wait()
    wt_v[dim:2 * dim, :] = wqkv_v[:, 2 * dim:3 * dim].T
    w_copy(1).wait()

    def project(i, carry):
        x_copy(i).wait()
        rows = pl.ds(pl.multiple_of(i * TQ, TQ), TQ)
        xn = _layernorm(x_v[rows, :].astype(F32))
        k = _pack(_dot(xn, wqkv_v[:, dim:2 * dim]))
        half = pl.ds(pl.multiple_of(i * (TQ // 2), TQ // 2), TQ // 2)
        for h in range(NUM_HEADS):
            group, lane = divmod(h * HEAD_DIM, 128)
            tile = k[:, group * 128:(group + 1) * 128]
            kk_v[h, half, :] = pltpu.roll(tile, 128 - lane, 1) if lane else tile
        qv = _dot(wt_v[...], xn, NT)
        qt_v[i] = (qv[0:dim] * q_scale).reshape(NUM_HEADS, HEAD_DIM, TQ)
        vt_v[i] = _pack(qv[dim:2 * dim]).reshape(NUM_HEADS, HEAD_DIM // 2, TQ)
        return carry

    lax.fori_loop(0, n_qb, project, 0)
    for copy in late:
        copy.start()

    gm = CK // 16 - 1

    def spread_keys(kb_ref, h, c, dims):
        r = (c * CK + gm * 16) // 2
        keys = _unpack(kk_v[h, r:r + 8, :]).astype(F32)
        out = []
        for d in dims:
            col = jnp.broadcast_to(keys[:, d:d + 1], (16, 128))
            kb_ref[c * HEAD_DIM + d] = col
            out.append(col)
        return out

    for c in range(n_ck):
        spread_keys(kba_v, 0, c, range(HEAD_DIM))

    hb = cfg["hb"]

    def attend(it, bad):
        always = lax.broadcasted_iota(I32, (8, 128), 0) + it >= 0
        zero = [lax.shift_right_logical(it + b, 12) if cfg["nocse"] else 0 for b in range(n_col)]
        per_head = n_qb * n_ck
        n_period = hb * per_head
        head = lambda t: it * hb + t // per_head
        block = lambda t: t % per_head // n_ck
        tables = [kba_v, kbb_v]
        scores, vpu_p, sums, outs = {}, {}, {}, {}

        def add_sum(t, b, p):
            key = (t // n_ck, b)
            sums[key] = sums[key] + p if key in sums else p

        def mxu_scores(lo, hi, ties):
            while lo < hi:
                end = min(hi, (lo // (n_ck * gm) + 1) * n_ck * gm)
                rows = []
                for n in range(lo, end):
                    t, j = divmod(n, gm)
                    r = (t % n_ck * CK + (gm - 1 - j) * 16) // 2
                    keys = kk_v[head(t), r:r + 8, :]
                    for value in ties.get(n, ()):
                        keys = jnp.where(always, keys, pltpu.bitcast(value, U32))
                    rows.append(keys)
                t = lo // gm
                keys = _unpack(jnp.concatenate(rows, axis=0))[:, 0:HEAD_DIM]
                s = _dot(keys, qt_v[block(t), head(t)])
                for i, n in enumerate(range(lo, end)):
                    scores[n] = s[i * 16:(i + 1) * 16]
                lo = end

        def vpu_scores(t, base):
            kb_ref = tables[t // per_head % 2]
            ties, cols = {}, []
            for b in range(n_col):
                lanes = slice(b * 128, (b + 1) * 128)
                s = _sum_tree(
                    [kb_ref[zero[b] + (t % n_ck * HEAD_DIM + d)]
                     * qt_v[block(t), head(t), d:d + 1, lanes] for d in range(HEAD_DIM)],
                    cfg["nacc"])
                p = jnp.exp2(s)
                part = p[0:8] + p[8:16]
                add_sum(t, b, part)
                ties.setdefault(base + cfg["tie"][b], []).append(part)
                cols.append(p)
            vpu_p[t] = jnp.concatenate(cols, axis=1)
            return ties

        def weigh_values(t, bad):
            tile = [vpu_p.pop(t)]
            for j in range(gm):
                p = jnp.exp2(scores.pop(t * gm + j))
                for b in range(n_col):
                    add_sum(t, b, p[0:8, b * 128:(b + 1) * 128] + p[8:16, b * 128:(b + 1) * 128])
                tile.append(p)
            c = t % n_ck
            lanes = slice(c % n_col * 128, (c % n_col + 1) * 128)
            values = _unpack(vt_v[c // n_col, head(t), :, lanes])
            o = _dot(values, jnp.concatenate(tile[::-1], axis=0))
            key = t // n_ck
            outs[key] = outs[key] + o if key in outs else o
            if c == n_ck - 1:
                total = jnp.concatenate([sums.pop((key, b)) for b in range(n_col)], axis=1)
                total = jnp.sum(total, axis=0, keepdims=True)
                o = outs.pop(key)
                safe = (total >= SUM_LO) & (total <= SUM_HI) & (jnp.abs(o) < jnp.inf)
                bad = jnp.where(safe, bad, 1.0)
                ot_v[block(t), head(t)] = o * (1.0 / total)
            return bad

        done = 0
        vlook = cfg["vlook"]
        per_step = n_ck * HEAD_DIM // per_head
        for t in range(-max(1, vlook), n_period):
            ties = vpu_scores(t + vlook, done) if 0 <= t + vlook < n_period else {}
            if 0 <= t + 1 < n_period:
                step = (t + 1) % per_head * per_step
                nxt = jnp.minimum(head(t + 1) + 1, NUM_HEADS - 1)
                cols = spread_keys(
                    tables[((t + 1) // per_head + 1) % 2], nxt, step // HEAD_DIM,
                    range(step % HEAD_DIM, step % HEAD_DIM + per_step))
                if cfg["kbtie"]:
                    for i, col in enumerate(cols):
                        ties.setdefault(done + (2, 4, 6, 6)[i], []).append(col[8:16])
            hi = min(n_period * gm, (t + 2) * gm + cfg["off"])
            if hi > done:
                mxu_scores(done, hi, ties)
                done = hi
            if t >= 0:
                bad = weigh_values(t, bad)
        return bad

    bad = lax.fori_loop(0, NUM_HEADS // hb, attend, jnp.zeros((HEAD_DIM, TQ), F32))

    @pl.when(jnp.max(bad) > 0.0)
    def _():
        def attend_shifted(it, carry):
            h, u = it // n_qb, it % n_qb
            keys = _unpack(kk_v[h])[:, 0:HEAD_DIM]
            values = jnp.concatenate([_unpack(vt_v[i, h]) for i in range(n_qb)], axis=1)
            for b in range(n_col):
                lanes = slice(b * 128, (b + 1) * 128)
                s = _dot(keys, qt_v[u, h, :, lanes])
                p = jnp.exp2(s - jnp.max(s, axis=0, keepdims=True))
                p = p * (1.0 / jnp.sum(p, axis=0, keepdims=True))
                ot_v[u, h, :, lanes] = _dot(values, p)
            return carry

        lax.fori_loop(0, NUM_HEADS * n_qb, attend_shifted, 0)

    late[0].wait()
    w_r = wr_ref[...].astype(F32).reshape(1, dim)

    def out_copy(i):
        rows = pl.ds(pl.multiple_of(i * TQ, TQ), TQ)
        return pltpu.make_async_copy(out_v.at[rows], out_hbm.at[0, rows], out_sem.at[i])

    lane_id = lax.broadcasted_iota(I32, (8, 128), 1)

    def finish(i, carry):
        rows = pl.ds(pl.multiple_of(i * TQ, TQ), TQ)
        attn = _dot(ot_v[i].reshape(dim, TQ).astype(BF16), wo_v[...], TN)
        h = _rnd(x_v[rows, :].astype(F32) + _rnd(attn))
        hn = _layernorm(h).astype(F32)
        h_v[rows, :] = h
        hn_v[rows, :] = hn
        out_v[rows, :] = (h + hn).astype(BF16)
        out_copy(i).start()
        r = jnp.sum(hn * w_r, axis=-1, keepdims=True)
        tile = jnp.zeros((8, 128), F32)
        for g in range(TQ // 8):
            tile = jnp.where(lane_id == g, r[g * 8:(g + 1) * 8], tile)
        return tuple(jnp.where(i == u, tile, old) for u, old in enumerate(carry))

    tiles = lax.fori_loop(0, n_qb, finish, tuple(jnp.zeros((8, 128), F32) for _ in range(n_qb)))

    score = _rnd(jnp.concatenate(tiles, axis=0))
    row = lax.broadcasted_iota(I32, score.shape, 0)
    lane = lax.broadcasted_iota(I32, score.shape, 1)
    token = (row // 8 * TQ + lane * 8 + row % 8).astype(F32)
    free = lane < TQ // 8
    rank = jnp.where(score == score, score, -jnp.inf)
    picked, gates = [], []
    for _ in range(CAPACITY):
        best = jnp.max(jnp.where(free, rank, -jnp.inf), keepdims=True)
        first = jnp.min(jnp.where(free & (rank == best), token, float(seq)), keepdims=True)
        chosen = free & (token == first)
        gates.append(jnp.sum(jnp.where(chosen, score, 0.0), keepdims=True))
        picked.append(jnp.min(first).astype(I32))
        free = free & (token != first)

    slot = lax.broadcasted_iota(I32, (16, dim), 0)
    x_sel = jnp.zeros((16, dim), F32)
    gate = jnp.zeros((16, 1), F32)
    for j in range(CAPACITY):
        x_sel = jnp.where(slot == j, hn_v[pl.ds(picked[j], 1), :], x_sel)
        gate = jnp.where(slot[:, 0:1] == j, gates[j], gate)
    x_sel = x_sel.astype(BF16)
    for copy in late[1:]:
        copy.wait()
    g = _rnd(_dot(x_sel, wg_v[...]))
    g = _rnd(g * _rnd(jax.nn.sigmoid(g)))
    u = _rnd(_dot(x_sel, wu_v[...]))
    y = _rnd(_dot((g * u).astype(BF16), wd_v[...]))
    y = _rnd(y * _rnd(jax.nn.sigmoid(gate)))

    for i in range(n_qb):
        out_copy(i).wait()
    bases = [pl.multiple_of(p // 16 * 16, 16) for p in picked]
    fixes = []
    for j, base in enumerate(bases):
        rows = pl.ds(base, 16)
        update = jnp.zeros((16, dim), F32)
        for k in range(CAPACITY):
            update = jnp.where(slot + base == picked[k], y[k:k + 1], update)
        fix_v[j] = (h_v[rows, :] + _rnd(hn_v[rows, :] + update)).astype(BF16)
        fixes.append(pltpu.make_async_copy(fix_v.at[j], out_hbm.at[0, rows], fix_sem.at[j]))
    distinct = bases[0] != bases[1]
    fixes[0].start()
    pl.when(distinct)(fixes[1].start)
    fixes[0].wait()
    pl.when(distinct)(fixes[1].wait)


@jax.jit
def pallas_sequential_preLN__mha_block__moe_arch_mod__prompt_kernel(
    A_x: jax.Array,
    A_wqkv: jax.Array,
    A_wo: jax.Array,
    B_x: jax.Array,
    B_w_r: jax.Array,
    B_w_gate: jax.Array,
    B_w_up: jax.Array,
    B_w_down: jax.Array,
):
    del B_x
    _, seq, dim = A_x.shape
    n_qb = seq // TQ
    hbm = pl.BlockSpec(memory_space=pl.ANY)
    table = pltpu.VMEM((seq // CK * HEAD_DIM, 16, 128), F32)
    return pl.pallas_call(
        functools.partial(_kernel, cfg=CFG),
        out_shape=jax.ShapeDtypeStruct(A_x.shape, A_x.dtype),
        in_specs=[hbm, hbm, hbm, pl.BlockSpec(memory_space=pltpu.VMEM), hbm, hbm, hbm],
        out_specs=hbm,
        scratch_shapes=[
            pltpu.VMEM((seq, dim), BF16),
            pltpu.VMEM(A_wqkv.shape, BF16),
            pltpu.VMEM(A_wo.shape, BF16),
            pltpu.VMEM(B_w_gate.shape, BF16),
            pltpu.VMEM(B_w_up.shape, BF16),
            pltpu.VMEM(B_w_down.shape, BF16),
            pltpu.VMEM((2 * dim, dim), BF16),
            pltpu.VMEM((n_qb, NUM_HEADS, HEAD_DIM, TQ), F32),
            pltpu.VMEM((NUM_HEADS, seq // 2, 128), U32),
            pltpu.VMEM((n_qb, NUM_HEADS, HEAD_DIM // 2, TQ), U32),
            table,
            table,
            pltpu.VMEM((n_qb, NUM_HEADS, HEAD_DIM, TQ), F32),
            pltpu.VMEM((seq, dim), F32),
            pltpu.VMEM((seq, dim), F32),
            pltpu.VMEM((seq, dim), BF16),
            pltpu.VMEM((CAPACITY, 16, dim), BF16),
            pltpu.SemaphoreType.DMA((n_qb + 7,)),
            pltpu.SemaphoreType.DMA((n_qb,)),
            pltpu.SemaphoreType.DMA((CAPACITY,)),
        ],
        compiler_params=pltpu.CompilerParams(vmem_limit_bytes=100 * 2**20),
        name="block",
    )(A_x, A_wqkv, A_wo, B_w_r, B_w_gate, B_w_up, B_w_down)
```

```python
import functools

import jax
import jax.numpy as jnp
import numpy as np
from jax import lax
from jax.experimental import pallas as pl
from jax.experimental.pallas import tpu as pltpu

F32, BF16, I32 = jnp.float32, jnp.bfloat16, jnp.int32

NUM_HEADS = 32
HEAD_DIM = 16
CAPACITY = 2
LN_EPS = 1e-5
LOG2E = float(np.log2(np.e))

TQ = 512
CK = 128
GROUP = 16
COLUMNS = TQ // 128
PER_TILE = 128 // HEAD_DIM
HALF = HEAD_DIM // 2
PRODUCTS = 7

SUM_LIMIT, VALUE_LIMIT = 2.0**30, 2.0**90

VECTOR_GROUPS = 22
PHASE = 10
LAG = 8
SPREAD_STEPS = (19, 36, 53, 70, 87, 104)
ORDERS = (
    ("b16 b7 b53 b42 a16 a7 a53 a42", ""),
    ("a16 a7 a53 a42 b16 b7 b53 b42", ""),
    ("b16 b7 b5 b3 b42 a16 a7 a5 a3 a42", ""),
    ("b16 b75 b3 b42 a16 a75 a3 a42", ""),
    ("b12 b67 b53 b4 a12 a67 a53 a4", ""),
    ("b16 b74 b53 b2 a16 a74 a53 a2", ""),
    ("a1 b16 b7 b53 b4 a6 a7 a53 a42 b2", "12"),
    ("a1 b16 b7 b53 b42 a67 a53 a42", "1"),
    ("b16 b7 b53 b4 a16 a7 a53 a42 b2", "2"),
    ("a1 b12 a26 b67 a74 b45 a53 b3", "1234567"),
)
ORDER_OF_GROUP = "99727599996997071898992952895955471299192826"
NUDGE_OF_STEP = (
    "6444444444444443335335444444444446666421523224444456444534444"
    "4552254553244664468775434442555544544434442444526755555534554"
    "6666444644444222653445444244445557422424444444444334244444444"
    "4475744444444112033444344454453464443455544347563544324224444"
)
GROUP_COST = 2 * (HALF * PRODUCTS + 2)

OUT_ROWS = 128
OUT_STOPS = (768, 1408, 1792, 2048)


def _dot(a, b, contract=((1,), (0,))):
    return lax.dot_general(a, b, (contract, ((), ())), preferred_element_type=F32)


def _rnd(x):
    return x.astype(BF16).astype(F32)


def _pack(x):
    return pltpu.bitcast(x.astype(BF16), I32)


def _unpack(x):
    return pltpu.bitcast(x, BF16)


def _lanes(b):
    return slice(b * 128, (b + 1) * 128)


def _start(*copies):
    for copy in copies:
        copy.start()


def _wait(*copies):
    for copy in copies:
        copy.wait()


def _center(x):
    centered = x - jnp.mean(x, axis=-1, keepdims=True)
    var = _rnd(_rnd(jnp.mean(centered * centered, axis=-1, keepdims=True)) + LN_EPS)
    std = _rnd(jnp.exp2(jnp.log(var) * (0.5 * LOG2E)))
    return centered, pltpu.reciprocal(std, approx=True)


def _vector_scores(key, query, order, emit):
    values, probs = {}, {}

    def product(block, j, start=None):
        sums = [] if start is None else [start]
        for d in range(HALF):
            term = key(block, j, d) * query(block, j, d)
            if len(sums) < 2:
                sums.append(term)
            else:
                sums[d % 2] = sums[d % 2] + term
        return sums[0] + sums[1]

    def finish(row, column, score):
        probs[row, column] = jnp.exp2(score)
        if (1 - row, column) in probs:
            upper, lower = probs[0, column], probs[1, column]
            emit(column, jnp.concatenate([upper, lower], axis=0), upper + lower)
        return score

    for step in order.split():
        block, names = "ab".index(step[0]), step[1:]
        v = values.setdefault(block, {})
        yield sum(HALF + 2 * (j == "3") for j in names)
        for j in names:
            if j == "1":
                v[j] = product(block, 0)
            elif j == "6":
                v[j] = product(block, 5, v["1"])
            elif j == "7":
                v[j] = product(block, 6, v["6"])
            elif j == "4":
                v[j] = finish(1, 2 * block, product(block, 3, v["7"]))
            elif j == "2":
                v[j] = finish(0, 2 * block, product(block, 1, v["1"]))
            elif j == "5":
                v[j] = product(block, 4)
            else:
                finish(1, 2 * block + 1, v["7"] + v["5"])
                v[j] = finish(0, 2 * block + 1, product(block, 2, v["6"] + v["5"]))
        yield [v[j] for j in names
               if j in "423" or j == names[-1] or (j == "7" and "4" not in names)]


class _Pacer:
    def __init__(self, steps, keep):
        self.steps, self.keep, self.spent = steps, keep, 0
        self.cost = next(steps, None)

    def advance(self, wanted):
        done = []
        while self.cost is not None and wanted():
            self.spent += self.cost
            done.extend(next(self.steps))
            self.cost = next(self.steps, None)
        return done

    def tie(self, words, budget):
        done = self.advance(lambda: self.spent + 0.2 * self.cost <= budget)
        for keep, value in zip(self.keep, done[-len(self.keep):]):
            words = jnp.where(keep, words, pltpu.bitcast(value, I32))
        return words


def _kernel(
    x_hbm, wqkv_hbm, wo_hbm, wr_hbm, wg_hbm, wu_hbm, wd_hbm,
    out_hbm,
    x_v, wqkv_v, wo_v, wr_v, wg_v, wu_v, wd_v,
    qt_v, qs_v, kk_v, ks_v, vt_v, even_v, odd_v, ot_v,
    h_v, hn_v, out_v, y_v, fix_v, picked_s,
    in_sem, out_sem, fix_sem,
):
    seq, dim = x_v.shape
    n_blocks, n_chunks, half = seq // TQ, seq // CK, dim // 2

    places = [divmod(place, 8) for place in range(n_chunks * 8)]
    on_vector = [places[(k * len(places) + PHASE) // VECTOR_GROUPS] for k in range(VECTOR_GROUPS)]
    first_key = lambda chunk, place: chunk * CK + (7 - place) * GROUP
    vector_keys = [first_key(*place) for place in on_vector]

    sems = iter(range(in_sem.shape[0]))
    copy_in = lambda src, dst: pltpu.make_async_copy(src, dst, in_sem.at[next(sems)])
    stops = (0, 256, 512, 1024, seq)
    x_copy = [copy_in(x_hbm.at[0, a:b], x_v.at[a:b]) for a, b in zip(stops, stops[1:])]
    stops = (0, dim, dim + half, 2 * dim, 3 * dim)
    wq_copy, wk_copy, wk_rest, wv_copy = (
        copy_in(wqkv_hbm.at[:, a:b], wqkv_v.at[:, a:b]) for a, b in zip(stops, stops[1:]))
    late = [copy_in(wo_hbm, wo_v), copy_in(wr_hbm, wr_v.at[0:dim]), copy_in(wg_hbm, wg_v),
            copy_in(wu_hbm, wu_v), copy_in(wd_hbm, wd_v)]
    _start(x_copy[0], wk_copy, wk_rest, x_copy[1], x_copy[2], wq_copy, wv_copy, x_copy[3])

    normed = {}

    def normalize(lo, hi):
        for r in range(lo, hi, GROUP):
            normed[r] = _center(x_v[r:r + GROUP, :].astype(F32))
            hn_v[r:r + GROUP, :] = jnp.multiply(*normed[r])

    def project_keys(lo, hi, tiles=range(dim // 128), scale_late=True):
        w = wqkv_v[:, dim + tiles.start * 128:dim + tiles.stop * 128]
        if scale_late:
            centered, scale = (
                jnp.concatenate([normed[r][j] for r in range(lo, hi, GROUP)], axis=0) for j in (0, 1))
            keys = _dot(centered.astype(BF16), w) * scale
        else:
            keys = _dot(hn_v[lo:hi, :].astype(BF16), w)
        for r in range(lo, hi, GROUP):
            part = keys[r - lo:r - lo + GROUP]
            words = _pack(part)
            for g in tiles:
                lanes = _lanes(g - tiles.start)
                kk_v[g * PER_TILE // 2, r // 2:r // 2 + 8, :] = words[:, lanes]
                if r in vector_keys:
                    a11, a21 = part[0:8, lanes], part[8:16, lanes]
                    a12, a22 = (pltpu.roll(a, 128 - HALF, 1) for a in (a11, a21))
                    s1 = a21 + a22
                    s2 = s1 - a11
                    for j, a in enumerate((a11, a12, a12 - s2, a22, s1, s2, a11 - a21)):
                        ks_v[g, vector_keys.index(r) * PRODUCTS + j] = a

    def share_keys(lo, hi, tiles=range(dim // 128)):
        for r in range(lo, hi, GROUP):
            rows = slice(r // 2, r // 2 + 8)
            for g in tiles:
                first = g * PER_TILE // 2
                if r not in vector_keys:
                    for pair in range(1, PER_TILE // 2):
                        kk_v[first + pair, rows, :] = pltpu.roll(
                            kk_v[first, rows, :], 128 - 2 * pair * HEAD_DIM, 1)
                elif g == 0:
                    entry = vector_keys.index(r) * PRODUCTS
                    for e in range(entry, entry + PRODUCTS):
                        for d in range(HALF):
                            even_v[e * HALF + d] = jnp.broadcast_to(ks_v[0, e][:, d:d + 1], (8, 128))

    def weight_terms(j, factor):
        w = wqkv_v[:, j * dim:(j + 1) * dim].T.astype(F32)
        size = jnp.minimum(jnp.max(jnp.abs(w), axis=-1, keepdims=True), 2.0**100)
        exponent = pltpu.bitcast(jnp.broadcast_to(size, (dim, 128)), I32) & 0x7F800000
        w = w * jnp.concatenate([pltpu.bitcast(0x7F000000 - exponent, F32)] * (dim // 128), axis=1)
        a11, a12, a21, a22 = w[:half, :half], w[:half, half:], w[half:, :half], w[half:, half:]
        terms = (a11 + a22, a21 + a22, a11, a22, a11 + a12, a21 - a11, a12 - a22)
        return [a.astype(BF16) for a in terms], pltpu.bitcast(exponent, F32) * factor

    def token_terms(u):
        first, second = hn_v[u * TQ:(u + 1) * TQ, :], hn_v[(u + 1) * TQ:(u + 2) * TQ, :]
        b11, b21, b12, b22 = first[:, :half], first[:, half:], second[:, :half], second[:, half:]
        terms = (b11 + b22, b11, b12 - b22, b21 - b11, b22, b11 + b12, b21 + b22)
        return [b.astype(BF16) for b in terms]

    def project_transposed(weights, tokens, u, store, midway=lambda: None):
        terms, scale = weights
        product = lambda j: _dot(terms[j], tokens[j], ((1,), (1,)))

        def finish(row, column, block):
            heads = slice(row * NUM_HEADS // 2, (row + 1) * NUM_HEADS // 2)
            rows = scale[row * half:(row + 1) * half]
            store(u + column, heads, block * jnp.concatenate([rows] * COLUMNS, axis=1))

        m3, m5 = product(2), product(4)
        finish(0, 1, m5 + m3)
        m2, m4 = product(1), product(3)
        finish(1, 0, m4 + m2)
        rest1, rest2 = m4 - m5, m3 - m2
        m1 = product(0)
        finish(0, 0, product(6) + (m1 + rest1))
        midway()
        finish(1, 1, product(5) + (m1 + rest2))

    def store_queries(u, heads, q):
        q = q.reshape(-1, HEAD_DIM, TQ)
        qt_v[u][heads] = q
        for k in range(COLUMNS // 2):
            b11, b21 = q[:, 0:8, _lanes(2 * k)], q[:, 8:16, _lanes(2 * k)]
            b12, b22 = q[:, 0:8, _lanes(2 * k + 1)], q[:, 8:16, _lanes(2 * k + 1)]
            t1 = b12 - b11
            t2 = b22 - t1
            for j, t in enumerate((b21 - t2, t1, t2, b22 - b12)):
                qs_v[u][heads, j * 8:(j + 1) * 8, _lanes(k)] = t

    peak = [jnp.zeros((8, 128), F32)]

    def store_values(u, heads, v):
        for r in range(0, v.shape[0], 8):
            peak[0] = jnp.maximum(peak[0], functools.reduce(
                jnp.maximum, [jnp.abs(v[r:r + 8, _lanes(b)]) for b in range(COLUMNS)]))
        vt_v[u, heads] = _pack(v).reshape(-1, HALF, TQ)

    _wait(x_copy[0])
    normalize(0, 256)
    _wait(wk_copy)
    project_keys(0, 256, range(0, 2))
    _wait(wk_rest)
    project_keys(0, 192, range(2, 4))
    _wait(x_copy[1])
    normalize(256, 512)
    project_keys(192, 256, range(2, 4))
    project_keys(256, 448)
    _wait(x_copy[2])
    normalize(512, 1024)
    project_keys(448, 512)
    project_keys(512, 896)
    _wait(wq_copy)
    wq = weight_terms(0, HEAD_DIM**-0.5 * LOG2E)
    project_keys(896, 1024, scale_late=False)
    tokens = token_terms(0)
    project_transposed(
        wq, tokens, 0, store_queries, lambda: (_wait(x_copy[3], wv_copy), _start(*late)))
    wv = weight_terms(2, 1.0)
    normalize(1024, seq)
    project_transposed(wv, tokens, 0, store_values)
    tokens = token_terms(2)
    for lo in range(1024, seq, 256):
        project_keys(lo, lo + 256, scale_late=False)
    share_keys(0, seq)
    project_transposed(wq, tokens, 2, store_queries)
    project_transposed(wv, tokens, 2, store_values)
    risk = jnp.max(peak[0], axis=0, keepdims=True) * (SUM_LIMIT / VALUE_LIMIT)

    blocks = [(i, u) for i in range(2) for u in range(n_blocks)]
    mxu_groups = [(blk, *place) for blk in blocks for place in places if place not in on_vector]
    vector_groups = [(blk, *place) for blk in blocks for place in on_vector]
    last = {(blk, c): n for n, (blk, c, _) in enumerate(mxu_groups)}
    program, done = [], 0
    for (blk, c), n in last.items():
        stop = last[blk, c + 1] + 1 if c == n_chunks - 2 else min(len(mxu_groups), n + 1 + LAG)
        program += mxu_groups[done:stop] + [(blk, c)]
        done = stop
    period = len(program) // len(blocks)
    share = VECTOR_GROUPS * PRODUCTS * HALF // n_blocks
    tables = (even_v, odd_v)

    def attend(pair, risk):
        keep = [lax.broadcasted_iota(I32, (8, 128), 0) + pair >= -j for j in range(3)]
        zero = [lax.shift_right_logical(pair + j, 12) for j in range(4)]
        head = [2 * pair, 2 * pair + 1]
        tiles, sums, pending, scored = {}, {}, [], []

        def add_sum(blk, b, p):
            sums[blk, b] = sums[blk, b] + p if (blk, b) in sums else p

        def vector_scores():
            for v, ((i, u), c, place) in enumerate(vector_groups):
                columns = {}
                entry = v % VECTOR_GROUPS * PRODUCTS
                order, shared = ORDERS[int(ORDER_OF_GROUP[i * VECTOR_GROUPS + v % VECTOR_GROUPS])]

                def key(block, j, d):
                    at = zero[block * (str(j + 1) not in shared)]
                    return tables[i][at + ((entry + j) * HALF + d)]

                def query(block, j, d):
                    h = head[i] + zero[v % 4]
                    if j < 3:
                        r = d + HALF * (j > 0)
                        return qt_v[u][h, r:r + 1, _lanes(2 * block + (j == 2))]
                    r = d + HALF * (j - 3)
                    return qs_v[u][h, r:r + 1, _lanes(block)]

                def emit(b, p, total):
                    columns[b] = p
                    add_sum((i, u), b, total)
                    if len(columns) == COLUMNS:
                        tiles[(i, u), c, place] = jnp.concatenate(
                            [columns[j] for j in range(COLUMNS)], axis=1)

                yield from _vector_scores(key, query, order, emit)

        pacer = _Pacer(vector_scores(), keep)
        rate = len(vector_groups) * GROUP_COST / len(program)

        def paced(n, words):
            (i, u), step = blocks[n // period], n % period
            nudge = 4 * (int(NUDGE_OF_STEP[i * period + step]) - 4)
            words = pacer.tie(words, (n - 1) * rate + nudge)
            if step in SPREAD_STEPS:
                j, following = SPREAD_STEPS.index(step), head[i] + 1
                g = lax.shift_right_logical(following, 3) & (dim // 128 - 1)
                member = following & (PER_TILE - 1)
                recent = pltpu.bitcast(scored[min(-1, len(pending) - 10)], I32)
                lane = {}
                for job in range(u * share + j * share // len(SPREAD_STEPS),
                                 u * share + (j + 1) * share // len(SPREAD_STEPS)):
                    d, e = divmod(job, VECTOR_GROUPS * PRODUCTS)
                    if d not in lane:
                        lane[d] = jnp.where(keep[0], member * HEAD_DIM + d, recent)
                    tables[1 - i][e * HALF + d] = jnp.take_along_axis(
                        ks_v[g, e], lane[d], axis=1, mode="promise_in_bounds")
            return words

        def mxu_scores():
            if not pending:
                return
            i, u = blk = pending[0][0][0]
            keys = _unpack(jnp.concatenate([words for _, words in pending], axis=0))
            q = qt_v[u][head[i]]
            q = jnp.concatenate([jnp.zeros_like(q)] * i + [q], axis=0)
            p = jnp.exp2(_dot(keys[:, 0:q.shape[0]], q))
            for j, (group, _) in enumerate(pending):
                tiles[group] = part = p[j * GROUP:(j + 1) * GROUP]
                scored.append(part[0:8, 0:128])
                for b in range(COLUMNS):
                    add_sum(blk, b, part[0:8, _lanes(b)] + part[8:16, _lanes(b)])
            pending.clear()

        for n, step in enumerate(program):
            blk, c = step[:2]
            i, u = blk
            if len(step) == 3:
                if pending and pending[0][0][0] != blk:
                    mxu_scores()
                r = first_key(*step[1:]) // 2
                pending.append((step, paced(n, kk_v[pair, r:r + 8, :])))
                continue
            mxu_scores()
            pacer.advance(lambda: any((blk, c, place) not in tiles for place in range(8)))
            values = _unpack(paced(n, vt_v[c // COLUMNS, head[i], :, _lanes(c % COLUMNS)]))
            o = _dot(values, jnp.concatenate(
                [tiles.pop((blk, c, place)) for place in range(7, -1, -1)], axis=0))
            if c > 0:
                o = o + ot_v[u, head[i] + zero[c % 2]]
            if c < n_chunks - 1:
                ot_v[u, head[i] + zero[c % 2]] = o
                continue
            total = jnp.concatenate([sums.pop((blk, b)) for b in range(COLUMNS)], axis=1)
            total = jnp.sum(total, axis=0, keepdims=True)
            inverse = pltpu.reciprocal(total, approx=True)
            ot_v[u, head[i]] = o * inverse
            for b in range(COLUMNS):
                risk = jnp.maximum(risk, jnp.maximum(total[:, _lanes(b)], inverse[:, _lanes(b)]))
        return risk

    risk = lax.fori_loop(0, NUM_HEADS // 2, attend, risk)

    _wait(*late)
    w_r = wr_v[0:dim].astype(F32).reshape(1, dim)
    lane_id = lax.broadcasted_iota(I32, (8, 128), 1)
    slot = lax.broadcasted_iota(I32, (GROUP, dim), 0)

    def project_out(heads):
        return _dot(heads.reshape(dim, OUT_ROWS).astype(BF16).T, wo_v[...])

    def residual(rows, attn):
        h = x_v[rows, :].astype(F32) + attn
        hn = jnp.multiply(*_center(h))
        h_v[rows, :] = h
        hn_v[rows, :] = hn
        out_v[rows, :] = (h + hn).astype(BF16)
        return jnp.sum(hn * w_r, axis=-1, keepdims=True)

    def record(tile, r, lane):
        for g in range(r.shape[0] // 8):
            tile = jnp.where(lane_id == lane + g, r[g * 8:(g + 1) * 8], tile)
        return tile

    def best_tokens(score):
        rank = _rnd(jnp.concatenate(score, axis=0))
        row = lax.broadcasted_iota(I32, rank.shape, 0)
        token = row // 8 * 1024 + lax.broadcasted_iota(I32, rank.shape, 1) * 8 + row % 8
        huge, tiny = float(jnp.finfo(BF16).max), float(jnp.finfo(BF16).tiny)
        rank = jnp.clip(jnp.where(rank == rank, rank, -huge), -huge, huge)
        rank = jnp.where(jnp.abs(rank) < tiny, tiny, rank)
        key = pltpu.bitcast(
            pltpu.bitcast(rank, I32) | jnp.where(rank > 0.0, seq - 1 - token, token), F32)
        picked = []
        for _ in range(CAPACITY):
            best = jnp.broadcast_to(jnp.max(key, keepdims=True), (8, 128))
            low = pltpu.bitcast(best, I32) & (seq - 1)
            picked.append(jnp.where(best > 0.0, seq - 1 - low, low)[0, 0])
            key = jnp.where(key == best[0:1], -jnp.inf, key)
        return picked

    def swiglu(picked):
        x_sel = jnp.zeros((GROUP, dim), F32)
        for j in range(CAPACITY):
            x_sel = jnp.where(slot == j, hn_v[pl.ds(picked[j], 1), :], x_sel)
        gate = jax.nn.sigmoid(jnp.sum(x_sel[0:8] * w_r, axis=-1, keepdims=True))
        x_sel = x_sel.astype(BF16)
        g = _dot(x_sel, wg_v[...])[0:8]
        u = _dot(x_sel, wu_v[...])[0:8]
        y_v[...] = _dot((g * jax.nn.sigmoid(g) * u).astype(BF16), wd_v[...]) * gate

    def heads_of(lo):
        return ot_v[lo // TQ, :, :, lo % TQ:lo % TQ + OUT_ROWS]

    score = [jnp.full((8, 128), -jnp.inf, F32) for _ in range(seq // 1024)]
    out_copies = []
    following = project_out(heads_of(0))
    for lo in range(0, seq, OUT_ROWS):
        hi, attn = lo + OUT_ROWS, following
        if hi < seq:
            following = project_out(heads_of(hi))
        if hi + OUT_ROWS == seq:
            guess = best_tokens(score)
        if hi == seq:
            swiglu(guess)
        r = residual(slice(lo, hi), attn)
        score[lo // 1024] = record(score[lo // 1024], r, lo // 8 % 128)
        if hi in OUT_STOPS:
            rows = slice((0, *OUT_STOPS)[len(out_copies)], hi)
            out_copies.append(pltpu.make_async_copy(
                out_v.at[rows], out_hbm.at[0, rows], out_sem.at[len(out_copies)]))
            out_copies[-1].start()
    for j, token in enumerate(best_tokens(score)):
        picked_s[j] = token
    unsafe = jnp.min(jnp.where(risk <= SUM_LIMIT, 1.0, 0.0)) == 0.0
    _wait(*out_copies)

    @pl.when(unsafe)
    def _():
        for u in range(n_blocks):
            ot_v[u] = qt_v[u][...]

        def redo(t, score):
            u, lanes = t // COLUMNS, pl.ds(pl.multiple_of(t % COLUMNS * 128, 128), 128)

            @pl.loop(0, NUM_HEADS)
            def _(h):
                member = lax.broadcasted_iota(I32, (128, 128), 0) // HEAD_DIM == h % PER_TILE
                q = jnp.concatenate([ot_v[u, h, :, lanes]] * PER_TILE, axis=0)
                s = _dot(_unpack(kk_v[(h - h % PER_TILE) // 2]), jnp.where(member, q, 0.0))
                p = jnp.exp2(s - jnp.max(s, axis=0, keepdims=True))
                values = jnp.concatenate([_unpack(vt_v[i, h]) for i in range(n_blocks)], axis=1)
                ot_v[u, h, :, lanes] = _dot(values, p * (1.0 / jnp.sum(p, axis=0, keepdims=True)))

            rows = pl.ds(pl.multiple_of(t * OUT_ROWS, OUT_ROWS), OUT_ROWS)
            r = residual(rows, project_out(ot_v[u, :, :, lanes]))
            return [record(tile, r, t * OUT_ROWS // 8 - i * 128) for i, tile in enumerate(score)]

        for j, token in enumerate(best_tokens(lax.fori_loop(0, seq // OUT_ROWS, redo, score))):
            picked_s[j] = token
        resend = pltpu.make_async_copy(out_v, out_hbm.at[0], out_sem.at[0])
        resend.start()
        resend.wait()

    picked = [picked_s[j] for j in range(CAPACITY)]

    @pl.when(unsafe | (picked[0] != guess[0]) | (picked[1] != guess[1]))
    def _():
        swiglu(picked)

    bases = [pl.multiple_of(p // GROUP * GROUP, GROUP) for p in picked]
    fixes = []
    for j, base in enumerate(bases):
        rows = pl.ds(base, GROUP)
        update = jnp.zeros((GROUP, dim), F32)
        for k in range(CAPACITY):
            update = jnp.where(slot + base == picked[k], y_v[k:k + 1, :], update)
        fix_v[j] = (h_v[rows, :] + (hn_v[rows, :] + update)).astype(BF16)
        fixes.append(pltpu.make_async_copy(fix_v.at[j], out_hbm.at[0, rows], fix_sem.at[j]))
    distinct = bases[0] != bases[1]
    fixes[0].start()
    pl.when(distinct)(fixes[1].start)
    fixes[0].wait()
    pl.when(distinct)(fixes[1].wait)


@jax.jit
def pallas_sequential_preLN__mha_block__moe_arch_mod__prompt_kernel(
    A_x: jax.Array,
    A_wqkv: jax.Array,
    A_wo: jax.Array,
    B_x: jax.Array,
    B_w_r: jax.Array,
    B_w_gate: jax.Array,
    B_w_up: jax.Array,
    B_w_down: jax.Array,
):
    del B_x
    _, seq, dim = A_x.shape
    n_blocks = seq // TQ
    hbm = pl.BlockSpec(memory_space=pl.ANY)
    table = pltpu.VMEM((VECTOR_GROUPS * PRODUCTS * HALF, 8, 128), F32)
    return pl.pallas_call(
        _kernel,
        out_shape=jax.ShapeDtypeStruct(A_x.shape, A_x.dtype),
        in_specs=[hbm] * 7,
        out_specs=hbm,
        scratch_shapes=[
            pltpu.VMEM((seq, dim), BF16),
            pltpu.VMEM(A_wqkv.shape, BF16),
            pltpu.VMEM(A_wo.shape, BF16),
            pltpu.VMEM((8192,), BF16),
            pltpu.VMEM(B_w_gate.shape, BF16),
            pltpu.VMEM(B_w_up.shape, BF16),
            pltpu.VMEM(B_w_down.shape, BF16),
            [pltpu.VMEM((NUM_HEADS, HEAD_DIM, TQ), F32)] * n_blocks,
            [pltpu.VMEM((NUM_HEADS, 2 * HEAD_DIM, TQ // 2), F32)] * n_blocks,
            pltpu.VMEM((NUM_HEADS // 2, seq // 2, 128), I32),
            pltpu.VMEM((dim // 128, pl.cdiv(VECTOR_GROUPS * PRODUCTS, 4) * 4, 8, 128), F32),
            pltpu.VMEM((n_blocks, NUM_HEADS, HALF, TQ), I32),
            table,
            table,
            pltpu.VMEM((n_blocks, NUM_HEADS, HEAD_DIM, TQ), F32),
            pltpu.VMEM((seq, dim), F32),
            pltpu.VMEM((seq, dim), F32),
            pltpu.VMEM((seq, dim), BF16),
            pltpu.VMEM((8, dim), F32),
            pltpu.VMEM((CAPACITY, GROUP, dim), BF16),
            pltpu.SMEM((CAPACITY,), I32),
            pltpu.SemaphoreType.DMA((13,)),
            pltpu.SemaphoreType.DMA((len(OUT_STOPS),)),
            pltpu.SemaphoreType.DMA((CAPACITY,)),
        ],
        compiler_params=pltpu.CompilerParams(vmem_limit_bytes=100 * 2**20),
        name="block",
    )(A_x, A_wqkv, A_wo, B_w_r, B_w_gate, B_w_up, B_w_down)
```

```python
import functools

import jax
import jax.numpy as jnp
import numpy as np
from jax import lax
from jax.experimental import pallas as pl
from jax.experimental.pallas import tpu as pltpu

F32, BF16, I32 = jnp.float32, jnp.bfloat16, jnp.int32

NUM_HEADS = 32
HEAD_DIM = 16
CAPACITY = 2
LN_EPS = 1e-5
LOG2E = float(np.log2(np.e))

TQ = 512
CK = 128
GROUP = 16
COLUMNS = TQ // 128
PER_TILE = 128 // HEAD_DIM
HALF = HEAD_DIM // 2
PRODUCTS = 7

SUM_LIMIT, VALUE_LIMIT = 2.0**60, 2.0**60

VECTOR_PLACES = (
    0, 6, 11, 16, 23, 29, 37, 41, 47, 52, 57, 64, 69, 76, 81, 86, 93, 99, 105, 110, 115, 119)
VECTOR_GROUPS = len(VECTOR_PLACES)
LAG = 8
HELD_STEP = 2
SPREAD_STEPS = (19, 39, 53, 70, 87, 103)
ORDERS = (
    ("b16 b7 b53 b42 a16 a7 a53 a42", ""),
    ("a16 a7 a53 a42 b16 b7 b53 b42", ""),
    ("b16 b7 b5 b3 b42 a16 a7 a5 a3 a42", ""),
    ("b16 b75 b3 b42 a16 a75 a3 a42", ""),
    ("b12 b67 b53 b4 a12 a67 a53 a4", ""),
    ("b16 b74 b53 b2 a16 a74 a53 a2", ""),
    ("a1 b16 b7 b53 b4 a6 a7 a53 a42 b2", "12"),
    ("a1 b16 b7 b53 b42 a67 a53 a42", "1"),
    ("b16 b7 b53 b4 a16 a7 a53 a42 b2", "2"),
    ("a1 b12 a26 b67 a74 b45 a53 b3", "1234567"),
)
ORDER_OF_GROUP = (
    "9974759999699707189896697475999939970718989639747599996997771898969674759999699707189796"
    "2942995955470343292946590209595542834389299669420959054153428929962942008905970341892996"
)
NUDGE_OF_STEP = (
    "3033445421446443335335323344555668656421523224444454244534444"
    "4552054774354664368776764545555546544434220223406535557757886"
    "6366445421446443335335323344555668656421523224444454244534444"
    "4552054774376884368776764545555546544454220223406424455424564"
    "3033445421446443335335323344553668656421523224444454244534444"
    "4552054774364664368776764545555546544434220223407545555535662"
    "3032445421446443335335323344555668656421523224444454244534444"
    "4552054763354664368765764545555546544433220123406535555535664"
    "6666474644144222600202111244445768433414444443346777444447783"
    "0033944445774443203466565665210253335579862236252877657565545"
    "6666474644124222520414111244445768432314444443345666444547783"
    "0023944447774443203444343465210253335579662236252878657665445"
    "6666252444144222731512122244445768432314444443346777444547783"
    "0023944447774453203444343465110253335578862236252877657665445"
    "6666494644144222620412111244445768654514444221145657555547783"
    "0023944448873333203444343465210253335579862236252877657665445"
)
GROUP_COST = 2 * (HALF * PRODUCTS + 2)

OUT_ROWS = 128
OUT_STOPS = (768, 1408, 1792, 2048)


def _dot(a, b, contract=((1,), (0,))):
    return lax.dot_general(a, b, (contract, ((), ())), preferred_element_type=F32)


def _rnd(x):
    return x.astype(BF16).astype(F32)


def _pack(x):
    return pltpu.bitcast(x.astype(BF16), I32)


def _unpack(x):
    return pltpu.bitcast(x, BF16)


def _lanes(b):
    return slice(b * 128, (b + 1) * 128)


def _start(*copies):
    for copy in copies:
        copy.start()


def _wait(*copies):
    for copy in copies:
        copy.wait()


def _center(x):
    centered = x - jnp.mean(x, axis=-1, keepdims=True)
    var = _rnd(_rnd(jnp.mean(centered * centered, axis=-1, keepdims=True)) + LN_EPS)
    std = _rnd(jnp.exp2(jnp.log(var) * (0.5 * LOG2E)))
    return centered, pltpu.reciprocal(std, approx=True)


def _vector_scores(key, query, order, emit):
    values, probs = {}, {}

    def product(block, j, start=None):
        sums = [] if start is None else [start]
        for d in range(HALF):
            term = key(block, j, d) * query(block, j, d)
            if len(sums) < 2:
                sums.append(term)
            else:
                sums[d % 2] = sums[d % 2] + term
        return sums[0] + sums[1]

    def finish(row, column, score):
        probs[row, column] = jnp.exp2(score)
        if (1 - row, column) in probs:
            upper, lower = probs[0, column], probs[1, column]
            emit(column, jnp.concatenate([upper, lower], axis=0), upper + lower)
        return score

    for step in order.split():
        block, names = "ab".index(step[0]), step[1:]
        v = values.setdefault(block, {})
        yield sum(HALF + 2 * (j == "3") for j in names)
        for j in names:
            if j == "1":
                v[j] = product(block, 0)
            elif j == "6":
                v[j] = product(block, 5, v["1"])
            elif j == "7":
                v[j] = product(block, 6, v["6"])
            elif j == "4":
                v[j] = finish(1, 2 * block, product(block, 3, v["7"]))
            elif j == "2":
                v[j] = finish(0, 2 * block, product(block, 1, v["1"]))
            elif j == "5":
                v[j] = product(block, 4)
            else:
                finish(1, 2 * block + 1, v["7"] + v["5"])
                v[j] = finish(0, 2 * block + 1, product(block, 2, v["6"] + v["5"]))
        yield [v[j] for j in names
               if j in "423" or j == names[-1] or (j == "7" and "4" not in names)]


class _Pacer:
    def __init__(self, steps, keep):
        self.steps, self.keep, self.spent = steps, keep, 0
        self.cost = next(steps, None)

    def advance(self, wanted):
        done = []
        while self.cost is not None and wanted():
            self.spent += self.cost
            done.extend(next(self.steps))
            self.cost = next(self.steps, None)
        return done

    def tie(self, words, budget):
        done = self.advance(lambda: self.spent + 0.2 * self.cost <= budget)
        for keep, value in zip(self.keep, done[-len(self.keep):]):
            words = jnp.where(keep, words, pltpu.bitcast(value, I32))
        return words


def _kernel(
    x_hbm, wqkv_hbm, wo_hbm, wr_hbm, wg_hbm, wu_hbm, wd_hbm,
    out_hbm,
    x_v, wqkv_v, wo_v, wr_v, wg_v, wu_v, wd_v,
    qt_v, qs_v, kk_v, ks_v, vt_v, even_v, odd_v, held_v, acc_v, ot_v,
    h_v, hn_v, out_v, y_v, fix_v, picked_s,
    sems,
):
    seq, dim = x_v.shape
    n_blocks, n_chunks, half = seq // TQ, seq // CK, dim // 2

    places = [divmod(place, 8) for place in range(n_chunks * 8)]
    on_vector = [places[place] for place in VECTOR_PLACES]
    first_key = lambda chunk, place: chunk * CK + (7 - place) * GROUP
    vector_keys = [first_key(*place) for place in on_vector]

    copy = lambda src, dst, sem: pltpu.make_async_copy(src, dst, sems.at[sem])
    stops = (0, 256, 512, 1024, seq)
    x_copy = [copy(x_hbm.at[0, a:b], x_v.at[a:b], sem)
              for sem, (a, b) in enumerate(zip(stops, stops[1:]))]
    stops = (0, dim, dim + half, 2 * dim, 3 * dim)
    wq_copy, wk_copy, wk_rest, wv_copy = (
        copy(wqkv_hbm.at[:, a:b], wqkv_v.at[:, a:b], sem)
        for sem, a, b in zip((4, 5, 6, 3), stops, stops[1:]))
    late = [copy(wo_hbm, wo_v, 0), copy(wr_hbm, wr_v.at[0:dim], 0), copy(wg_hbm, wg_v, 0),
            copy(wu_hbm, wu_v, 0), copy(wd_hbm, wd_v, 0)]
    _start(x_copy[0], wk_copy, wk_rest, x_copy[1], x_copy[2], wq_copy, wv_copy, x_copy[3])

    normed = {}

    def normalize(lo, hi):
        for r in range(lo, hi, GROUP):
            normed[r] = _center(x_v[r:r + GROUP, :].astype(F32))
            hn_v[r:r + GROUP, :] = jnp.multiply(*normed[r])

    def project_keys(lo, hi, tiles=range(dim // 128), scale_late=True):
        w = wqkv_v[:, dim + tiles.start * 128:dim + tiles.stop * 128]
        if scale_late:
            centered, scale = (
                jnp.concatenate([normed[r][j] for r in range(lo, hi, GROUP)], axis=0) for j in (0, 1))
            keys = _dot(centered.astype(BF16), w) * scale
        else:
            keys = _dot(hn_v[lo:hi, :].astype(BF16), w)
        for r in range(lo, hi, GROUP):
            part = keys[r - lo:r - lo + GROUP]
            words = _pack(part)
            for g in tiles:
                lanes = _lanes(g - tiles.start)
                kk_v[g * PER_TILE // 2, r // 2:r // 2 + 8, :] = words[:, lanes]
                if r in vector_keys:
                    a11, a21 = part[0:8, lanes], part[8:16, lanes]
                    a12, a22 = (pltpu.roll(a, 128 - HALF, 1) for a in (a11, a21))
                    s1 = a21 + a22
                    s2 = s1 - a11
                    for j, a in enumerate((a11, a12, a12 - s2, a22, s1, s2, a11 - a21)):
                        ks_v[g, vector_keys.index(r) * PRODUCTS + j] = a

    def share_keys(lo, hi, tiles=range(dim // 128)):
        for r in range(lo, hi, GROUP):
            rows = slice(r // 2, r // 2 + 8)
            for g in tiles:
                first = g * PER_TILE // 2
                if r not in vector_keys:
                    for pair in range(1, PER_TILE // 2):
                        kk_v[first + pair, rows, :] = pltpu.roll(
                            kk_v[first, rows, :], 128 - 2 * pair * HEAD_DIM, 1)
                elif g == 0:
                    entry = vector_keys.index(r) * PRODUCTS
                    for e in range(entry, entry + PRODUCTS):
                        for d in range(HALF):
                            even_v[e * HALF + d] = jnp.broadcast_to(ks_v[0, e][:, d:d + 1], (8, 128))

    def weight_terms(j, factor):
        w = wqkv_v[:, j * dim:(j + 1) * dim].T.astype(F32)
        size = jnp.minimum(jnp.max(jnp.abs(w), axis=-1, keepdims=True), 2.0**100)
        exponent = pltpu.bitcast(jnp.broadcast_to(size, (dim, 128)), I32) & 0x7F800000
        w = w * jnp.concatenate([pltpu.bitcast(0x7F000000 - exponent, F32)] * (dim // 128), axis=1)
        a11, a12, a21, a22 = w[:half, :half], w[:half, half:], w[half:, :half], w[half:, half:]
        terms = (a11 + a22, a21 + a22, a11, a22, a11 + a12, a21 - a11, a12 - a22)
        return [a.astype(BF16) for a in terms], pltpu.bitcast(exponent, F32) * factor

    def token_terms(u):
        first, second = hn_v[u * TQ:(u + 1) * TQ, :], hn_v[(u + 1) * TQ:(u + 2) * TQ, :]
        b11, b21, b12, b22 = first[:, :half], first[:, half:], second[:, :half], second[:, half:]
        terms = (b11 + b22, b11, b12 - b22, b21 - b11, b22, b11 + b12, b21 + b22)
        return [b.astype(BF16) for b in terms]

    def project_transposed(weights, tokens, u, store, midway=lambda: None):
        terms, scale = weights
        product = lambda j: _dot(terms[j], tokens[j], ((1,), (1,)))

        def finish(row, column, block):
            heads = slice(row * NUM_HEADS // 2, (row + 1) * NUM_HEADS // 2)
            rows = scale[row * half:(row + 1) * half]
            store(u + column, heads, block * jnp.concatenate([rows] * COLUMNS, axis=1))

        m3, m5 = product(2), product(4)
        finish(0, 1, m5 + m3)
        m2, m4 = product(1), product(3)
        finish(1, 0, m4 + m2)
        rest1, rest2 = m4 - m5, m3 - m2
        m1 = product(0)
        finish(0, 0, product(6) + (m1 + rest1))
        midway()
        finish(1, 1, product(5) + (m1 + rest2))

    def store_queries(u, heads, q):
        q = q.reshape(-1, HEAD_DIM, TQ)
        qt_v[u][heads] = q
        for k in range(COLUMNS // 2):
            b11, b21 = q[:, 0:8, _lanes(2 * k)], q[:, 8:16, _lanes(2 * k)]
            b12, b22 = q[:, 0:8, _lanes(2 * k + 1)], q[:, 8:16, _lanes(2 * k + 1)]
            t1 = b12 - b11
            t2 = b22 - t1
            for j, t in enumerate((b21 - t2, t1, t2, b22 - b12)):
                qs_v[u][heads, j * 8:(j + 1) * 8, _lanes(k)] = t

    def store_values(u, heads, v):
        vt_v[u, heads] = _pack(v).reshape(-1, HALF, TQ)

    _wait(x_copy[0])
    normalize(0, 256)
    _wait(wk_copy)
    project_keys(0, 256, range(0, 2))
    _wait(wk_rest)
    project_keys(0, 192, range(2, 4))
    _wait(x_copy[1])
    normalize(256, 512)
    project_keys(192, 256, range(2, 4))
    project_keys(256, 384)
    _wait(x_copy[2])
    normalize(512, 1024)
    project_keys(384, 512)
    project_keys(512, 896)
    _wait(wq_copy)
    wq = weight_terms(0, HEAD_DIM**-0.5 * LOG2E)
    project_keys(896, 1024, scale_late=False)
    tokens = token_terms(0)
    project_transposed(
        wq, tokens, 0, store_queries, lambda: (_wait(x_copy[3], wv_copy), _start(*late)))
    wv = weight_terms(2, 1.0)
    normalize(1024, seq)
    project_transposed(wv, tokens, 0, store_values)
    tokens = token_terms(2)
    for lo in range(1024, seq, TQ):
        project_keys(lo, lo + TQ, scale_late=False)
    share_keys(0, seq)
    project_transposed(wv, tokens, 2, store_values)
    project_transposed(wq, tokens, 2, store_queries)
    held_v[...] = jnp.zeros(held_v.shape, F32)
    risk = jnp.max(wv[1], axis=0, keepdims=True) * (4 * dim * SUM_LIMIT / VALUE_LIMIT)

    blocks = [(i, u) for i in range(2) for u in range(n_blocks)]
    mxu_groups = [(blk, *place) for blk in blocks for place in places if place not in on_vector]
    vector_groups = [(blk, *place) for blk in blocks for place in on_vector]
    last = {(blk, c): n for n, (blk, c, _) in enumerate(mxu_groups)}
    program, done = [], 0
    for (blk, c), n in last.items():
        stop = min(len(mxu_groups), n + 1 + LAG)
        if c == n_chunks - 2:
            stop = last[blk, c + 1] + 1
        program += mxu_groups[done:stop] + [(blk, c)]
        done = stop
    period = len(program) // len(blocks)
    share = VECTOR_GROUPS * PRODUCTS * HALF // n_blocks
    tables = (even_v, odd_v)

    def weigh_held(h):
        values = _unpack(vt_v[n_blocks - 1, h, :, _lanes(COLUMNS - 1)])
        o = _dot(values, held_v[0:CK]) + held_v[CK:CK + HEAD_DIM]
        ot_v[n_blocks - 1, h] = o * held_v[CK + HEAD_DIM:CK + HEAD_DIM + 1]

    def attend(pair, risk):
        keep = [lax.broadcasted_iota(I32, (8, 128), 0) + pair >= -j for j in range(3)]
        zero = [lax.shift_right_logical(pair + j, 12) for j in range(4)]
        head = [2 * pair, 2 * pair + 1]
        tiles, sums, pending, scored = {}, {}, [], []

        def add_sum(blk, b, p):
            sums[blk, b] = sums[blk, b] + p if (blk, b) in sums else p

        def vector_scores():
            for v, ((i, u), c, place) in enumerate(vector_groups):
                columns = {}
                entry = v % VECTOR_GROUPS * PRODUCTS
                order, shared = ORDERS[int(ORDER_OF_GROUP[v])]

                def key(block, j, d):
                    at = zero[block * (str(j + 1) not in shared)]
                    return tables[i][at + ((entry + j) * HALF + d)]

                def query(block, j, d):
                    h = head[i] + zero[v % 4]
                    if j < 3:
                        r = d + HALF * (j > 0)
                        return qt_v[u][h, r:r + 1, _lanes(2 * block + (j == 2))]
                    r = d + HALF * (j - 3)
                    return qs_v[u][h, r:r + 1, _lanes(block)]

                def emit(b, p, total):
                    columns[b] = p
                    add_sum((i, u), b, total)
                    if len(columns) == COLUMNS:
                        tiles[(i, u), c, place] = jnp.concatenate(
                            [columns[j] for j in range(COLUMNS)], axis=1)

                yield from _vector_scores(key, query, order, emit)

        pacer = _Pacer(vector_scores(), keep)
        rate = len(vector_groups) * GROUP_COST / len(program)

        def paced(n, words):
            (i, u), step = blocks[n // period], n % period
            nudge = 4 * (int(NUDGE_OF_STEP[n]) - 4)
            words = pacer.tie(words, (n - 1) * rate + nudge)
            if step in SPREAD_STEPS:
                j, following = SPREAD_STEPS.index(step), head[i] + 1
                g = lax.shift_right_logical(following, 3) & (dim // 128 - 1)
                member = following & (PER_TILE - 1)
                recent = pltpu.bitcast(scored[min(-1, len(pending) - 10)], I32)
                lane = {}
                for job in range(u * share + j * share // len(SPREAD_STEPS),
                                 u * share + (j + 1) * share // len(SPREAD_STEPS)):
                    d, e = divmod(job, VECTOR_GROUPS * PRODUCTS)
                    if d not in lane:
                        lane[d] = jnp.where(keep[0], member * HEAD_DIM + d, recent)
                    tables[1 - i][e * HALF + d] = jnp.take_along_axis(
                        ks_v[g, e], lane[d], axis=1, mode="promise_in_bounds")
            return words

        def mxu_scores():
            if not pending:
                return
            i, u = blk = pending[0][0][0]
            keys = _unpack(jnp.concatenate([words for _, words in pending], axis=0))
            q = qt_v[u][head[i]]
            q = jnp.concatenate([jnp.zeros_like(q)] * i + [q], axis=0)
            p = jnp.exp2(_dot(keys[:, 0:q.shape[0]], q))
            for j, (group, _) in enumerate(pending):
                tiles[group] = part = p[j * GROUP:(j + 1) * GROUP]
                scored.append(part[0:8, 0:128])
                for b in range(COLUMNS):
                    add_sum(blk, b, part[0:8, _lanes(b)] + part[8:16, _lanes(b)])
            pending.clear()

        for n, step in enumerate(program):
            if n == HELD_STEP:
                mxu_scores()
                weigh_held((head[0] - 1) & (NUM_HEADS - 1))
            blk, c = step[:2]
            i, u = blk
            if len(step) == 3:
                if pending and pending[0][0][0] != blk:
                    mxu_scores()
                r = first_key(*step[1:]) // 2
                pending.append((step, paced(n, kk_v[pair, r:r + 8, :])))
                continue
            mxu_scores()
            pacer.advance(lambda: any((blk, c, place) not in tiles for place in range(8)))
            p = jnp.concatenate([tiles.pop((blk, c, place)) for place in range(7, -1, -1)], axis=0)
            if n + 1 < len(program):
                o = _dot(_unpack(paced(n, vt_v[c // COLUMNS, head[i], :, _lanes(c % COLUMNS)])), p)
                if c > 0:
                    o = o + acc_v[zero[c % 2]]
                if n + 2 == len(program):
                    held_v[CK:CK + HEAD_DIM] = o
                    continue
                if c < n_chunks - 1:
                    acc_v[zero[c % 2]] = o
                    continue
            total = jnp.concatenate([sums.pop((blk, b)) for b in range(COLUMNS)], axis=1)
            total = jnp.sum(total, axis=0, keepdims=True)
            inverse = pltpu.reciprocal(total, approx=True)
            if n + 1 < len(program):
                ot_v[u, head[i]] = o * inverse
            else:
                held_v[0:CK] = p
                held_v[CK + HEAD_DIM:CK + HEAD_DIM + 8] = jnp.broadcast_to(inverse, (8, TQ))
            for b in range(COLUMNS):
                risk = jnp.maximum(risk, jnp.maximum(total[:, _lanes(b)], inverse[:, _lanes(b)]))
        return risk

    risk = lax.fori_loop(0, NUM_HEADS // 2, attend, risk)
    weigh_held(NUM_HEADS - 1)

    _wait(*late)
    w_r = wr_v[0:dim].astype(F32).reshape(1, dim)
    lane_id = lax.broadcasted_iota(I32, (8, 128), 1)
    slot = lax.broadcasted_iota(I32, (GROUP, dim), 0)

    def project_out(heads):
        return _dot(heads.reshape(dim, OUT_ROWS).astype(BF16).T, wo_v[...])

    def residual(rows, attn):
        h = x_v[rows, :].astype(F32) + attn
        hn = jnp.multiply(*_center(h))
        h_v[rows, :] = h
        hn_v[rows, :] = hn
        out_v[rows, :] = (h + hn).astype(BF16)
        return jnp.sum(hn * w_r, axis=-1, keepdims=True)

    def record(tile, r, lane):
        for g in range(r.shape[0] // 8):
            tile = jnp.where(lane_id == lane + g, r[g * 8:(g + 1) * 8], tile)
        return tile

    def best_tokens(score):
        rank = _rnd(jnp.concatenate(score, axis=0))
        row = lax.broadcasted_iota(I32, rank.shape, 0)
        token = row // 8 * 1024 + lax.broadcasted_iota(I32, rank.shape, 1) * 8 + row % 8
        huge, tiny = float(jnp.finfo(BF16).max), float(jnp.finfo(BF16).tiny)
        rank = jnp.clip(jnp.where(rank == rank, rank, -huge), -huge, huge)
        rank = jnp.where(jnp.abs(rank) < tiny, tiny, rank)
        key = pltpu.bitcast(
            pltpu.bitcast(rank, I32) | jnp.where(rank > 0.0, seq - 1 - token, token), F32)
        picked = []
        for _ in range(CAPACITY):
            best = jnp.broadcast_to(jnp.max(key, keepdims=True), (8, 128))
            low = pltpu.bitcast(best, I32) & (seq - 1)
            picked.append(jnp.where(best > 0.0, seq - 1 - low, low)[0, 0])
            key = jnp.where(key == best[0:1], -jnp.inf, key)
        return picked

    def swiglu(picked):
        x_sel = jnp.zeros((GROUP, dim), F32)
        for j in range(CAPACITY):
            x_sel = jnp.where(slot == j, hn_v[pl.ds(picked[j], 1), :], x_sel)
        gate = jax.nn.sigmoid(jnp.sum(x_sel[0:8] * w_r, axis=-1, keepdims=True))
        x_sel = x_sel.astype(BF16)
        g = _dot(x_sel, wg_v[...])[0:8]
        u = _dot(x_sel, wu_v[...])[0:8]
        y_v[...] = _dot((g * jax.nn.sigmoid(g) * u).astype(BF16), wd_v[...]) * gate

    def heads_of(lo):
        return ot_v[lo // TQ, :, :, lo % TQ:lo % TQ + OUT_ROWS]

    score = [jnp.full((8, 128), -jnp.inf, F32) for _ in range(seq // 1024)]
    out_copies = []
    following = project_out(heads_of(0))
    for lo in range(0, seq, OUT_ROWS):
        hi, attn = lo + OUT_ROWS, following
        if hi < seq:
            following = project_out(heads_of(hi))
        if hi + OUT_ROWS == seq:
            guess = best_tokens(score)
        if hi == seq:
            swiglu(guess)
        r = residual(slice(lo, hi), attn)
        score[lo // 1024] = record(score[lo // 1024], r, lo // 8 % 128)
        if hi in OUT_STOPS:
            rows = slice((0, *OUT_STOPS)[len(out_copies)], hi)
            out_copies.append(copy(out_v.at[rows], out_hbm.at[0, rows], 1))
            out_copies[-1].start()
    for j, token in enumerate(best_tokens(score)):
        picked_s[j] = token
    unsafe = jnp.min(jnp.where(risk <= SUM_LIMIT, 1.0, 0.0)) == 0.0
    _wait(*out_copies)

    @pl.when(unsafe)
    def _():
        for u in range(n_blocks):
            ot_v[u] = qt_v[u][...]

        def redo(t, score):
            u, lanes = t // COLUMNS, pl.ds(pl.multiple_of(t % COLUMNS * 128, 128), 128)

            @pl.loop(0, NUM_HEADS)
            def _(h):
                member = lax.broadcasted_iota(I32, (128, 128), 0) // HEAD_DIM == h % PER_TILE
                q = jnp.concatenate([ot_v[u, h, :, lanes]] * PER_TILE, axis=0)
                s = _dot(_unpack(kk_v[(h - h % PER_TILE) // 2]), jnp.where(member, q, 0.0))
                p = jnp.exp2(s - jnp.max(s, axis=0, keepdims=True))
                values = jnp.concatenate([_unpack(vt_v[i, h]) for i in range(n_blocks)], axis=1)
                ot_v[u, h, :, lanes] = _dot(values, p * (1.0 / jnp.sum(p, axis=0, keepdims=True)))

            rows = pl.ds(pl.multiple_of(t * OUT_ROWS, OUT_ROWS), OUT_ROWS)
            r = residual(rows, project_out(ot_v[u, :, :, lanes]))
            return [record(tile, r, t * OUT_ROWS // 8 - i * 128) for i, tile in enumerate(score)]

        for j, token in enumerate(best_tokens(lax.fori_loop(0, seq // OUT_ROWS, redo, score))):
            picked_s[j] = token
        resend = copy(out_v, out_hbm.at[0], 1)
        resend.start()
        resend.wait()

    picked = [picked_s[j] for j in range(CAPACITY)]

    @pl.when(unsafe | (picked[0] != guess[0]) | (picked[1] != guess[1]))
    def _():
        swiglu(picked)

    bases = [pl.multiple_of(p // GROUP * GROUP, GROUP) for p in picked]
    fixes = []
    for j, base in enumerate(bases):
        rows = pl.ds(base, GROUP)
        update = jnp.zeros((GROUP, dim), F32)
        for k in range(CAPACITY):
            update = jnp.where(slot + base == picked[k], y_v[k:k + 1, :], update)
        fix_v[j] = (h_v[rows, :] + (hn_v[rows, :] + update)).astype(BF16)
        fixes.append(copy(fix_v.at[j], out_hbm.at[0, rows], 2 + j))
    distinct = bases[0] != bases[1]
    fixes[0].start()
    pl.when(distinct)(fixes[1].start)
    fixes[0].wait()
    pl.when(distinct)(fixes[1].wait)


@jax.jit
def pallas_sequential_preLN__mha_block__moe_arch_mod__prompt_kernel(
    A_x: jax.Array,
    A_wqkv: jax.Array,
    A_wo: jax.Array,
    B_x: jax.Array,
    B_w_r: jax.Array,
    B_w_gate: jax.Array,
    B_w_up: jax.Array,
    B_w_down: jax.Array,
):
    del B_x
    _, seq, dim = A_x.shape
    n_blocks = seq // TQ
    hbm = pl.BlockSpec(memory_space=pl.ANY)
    table = pltpu.VMEM((VECTOR_GROUPS * PRODUCTS * HALF, 8, 128), F32)
    return pl.pallas_call(
        _kernel,
        out_shape=jax.ShapeDtypeStruct(A_x.shape, A_x.dtype),
        in_specs=[hbm] * 7,
        out_specs=hbm,
        scratch_shapes=[
            pltpu.VMEM((seq, dim), BF16),
            pltpu.VMEM(A_wqkv.shape, BF16),
            pltpu.VMEM(A_wo.shape, BF16),
            pltpu.VMEM((8192,), BF16),
            pltpu.VMEM(B_w_gate.shape, BF16),
            pltpu.VMEM(B_w_up.shape, BF16),
            pltpu.VMEM(B_w_down.shape, BF16),
            [pltpu.VMEM((NUM_HEADS, HEAD_DIM, TQ), F32)] * n_blocks,
            [pltpu.VMEM((NUM_HEADS, 2 * HEAD_DIM, TQ // 2), F32)] * n_blocks,
            pltpu.VMEM((NUM_HEADS // 2, seq // 2, 128), I32),
            pltpu.VMEM((dim // 128, pl.cdiv(VECTOR_GROUPS * PRODUCTS, 4) * 4, 8, 128), F32),
            pltpu.VMEM((n_blocks, NUM_HEADS, HALF, TQ), I32),
            table,
            table,
            pltpu.VMEM((CK + HEAD_DIM + 8, TQ), F32),
            pltpu.VMEM((1, HEAD_DIM, TQ), F32),
            pltpu.VMEM((n_blocks, NUM_HEADS, HEAD_DIM, TQ), F32),
            pltpu.VMEM((seq, dim), F32),
            pltpu.VMEM((seq, dim), F32),
            pltpu.VMEM((seq, dim), BF16),
            pltpu.VMEM((8, dim), F32),
            pltpu.VMEM((CAPACITY, GROUP, dim), BF16),
            pltpu.SMEM((CAPACITY,), I32),
            pltpu.SemaphoreType.DMA((7,)),
        ],
        compiler_params=pltpu.CompilerParams(vmem_limit_bytes=100 * 2**20),
        name="block",
    )(A_x, A_wqkv, A_wo, B_w_r, B_w_gate, B_w_up, B_w_down)
```
